```python
import os as _os
_os.environ.setdefault("JAX_PLATFORMS", "cpu")
import jax
import jax.numpy as jnp

def _softmax(x, axis=-1):
    return jax.nn.softmax(x, axis=axis)
def _gelu(x):
    return jax.nn.gelu(x, approximate=True)
def _silu(x):
    return jax.nn.silu(x)
def _sigmoid(x):
    return jax.nn.sigmoid(x)
def _layernorm(x, axis=-1, eps=1e-5):
    m = jnp.mean(x, axis=axis, keepdims=True)
    v = jnp.var(x, axis=axis, keepdims=True)
    return (x - m) / jnp.sqrt(v + eps)
def _scatter_add(tgt, idx, src, axis=0):
    return tgt.at[idx].add(src)
def _segment_sum(src, seg, n):
    return jax.ops.segment_sum(src, seg, n)
class _Rng:
    def __init__(self, key):
        self._k = key
    def _next(self):
        self._k, sub = jax.random.split(self._k)
        return sub
    def normal(self, shape):
        return jax.random.normal(self._next(), shape, dtype=jnp.bfloat16)
    def randint(self, lo, hi, shape):
        return jax.random.randint(self._next(), shape, lo, hi, dtype=jnp.int32)
    def uniform(self, shape, lo=0.0, hi=1.0):
        return jax.random.uniform(self._next(), shape, jnp.bfloat16, lo, hi)
    def permutation(self, n):
        return jax.random.permutation(self._next(), n)


kernel_name = 'standalone__mha_block_cached__near_ridge'

def setup_inputs():
    _rng = _Rng(jax.random.key(int.from_bytes(__import__("os").urandom(4), "little")))
    _w = (lambda a: (lambda t: t.astype(jnp.bfloat16) if jnp.issubdtype(t.dtype, jnp.floating) else t)(jnp.asarray(a)))
    B, Sq, D = 8, 112, 640
    H, Sk, Dh = 32, 512, 192
    return {
        "x": _w((lambda *s: _rng.normal(s) * 0.8)(B, Sq, D)),
        "k_cache": _w((lambda *s: _rng.normal(s) * 0.8)(B, H, Sk, Dh)),
        "v_cache": _w((lambda *s: _rng.normal(s) * 0.05)(B, H, Sk, Dh)),
        "wq": _w((lambda *s: _rng.normal(s) * 0.8)(D, H * Dh) * (D ** -0.5)),
        "wo": _w((lambda *s: _rng.normal(s) * 0.05)(H * Dh, D) * ((H * Dh) ** -0.5)),
    }

def reference(x, k_cache, v_cache, wq, wo):
    B, Sq, D = x.shape
    H, Dh = 32, 192
    q = (lambda x, *d: x.transpose(*d))((x @ wq).reshape(B, Sq, H, Dh), 0, 2, 1, 3)
    scores = jnp.einsum("bhqd,bhkd->bhqk", q, k_cache) * (Dh ** -0.5)
    p = _softmax(scores, axis=-1)
    o = jnp.einsum("bhqk,bhkd->bhqd", p, v_cache)
    return (lambda x, *d: x.transpose(*d))(o, 0, 2, 1, 3).reshape(B, Sq, H * Dh) @ wo
```

```python
import functools
import jax
import jax.numpy as jnp
from jax.experimental import pallas as pl
from jax.experimental.pallas import tpu as pltpu

U = 2
NSLOT = 4
LOG2E = 1.4426950408889634
F32 = jnp.float32
BF16 = jnp.bfloat16
NT = (((1,), (1,)), ((), ()))


def _log2(n):
    r = n.bit_length() - 1
    assert 1 << r == n
    return r


def _kernel(x_hbm, kt_hbm, vt_hbm, wq_hbm, wo_hbm, o_hbm,
            x_buf, wq_buf, wo_buf, k_buf, v_buf, p_buf, r_buf, acc, out_buf,
            sem_x, sem_wq, sem_wo, sem_k, sem_v, sem_o, *, U, NSLOT):
    B, Sq, D = x_hbm.shape
    _, H, Dh, Sk = kt_hbm.shape
    NP = H // 2
    GP = B // U
    NG = NP * GP
    LGP = _log2(GP)
    M = U * Sq
    W = 2 * Dh
    qscale = (Dh ** -0.5) * LOG2E

    def hp_of(g): return g >> LGP
    def gi_of(g): return g & (GP - 1)

    def kv_copy(hbm, buf, sem, g):
        slot = g & (NSLOT - 1)
        return pltpu.make_async_copy(hbm.at[pl.ds(gi_of(g) * U, U), pl.ds(2 * hp_of(g), 2)], buf.at[slot], sem.at[slot])

    def k_copy(g): return kv_copy(kt_hbm, k_buf, sem_k, g)
    def v_copy(g): return kv_copy(vt_hbm, v_buf, sem_v, g)
    def wq_copy(hp):
        return pltpu.make_async_copy(wq_hbm.at[:, pl.ds(hp * W, W)], wq_buf.at[hp & 1], sem_wq.at[hp & 1])
    def wo_copy(hp):
        return pltpu.make_async_copy(wo_hbm.at[pl.ds(hp * W, W), :], wo_buf.at[hp & 1], sem_wo.at[hp & 1])
    def x_copy(gi):
        return pltpu.make_async_copy(x_hbm.at[pl.ds(gi * U, U)], x_buf.at[pl.ds(gi * U, U)], sem_x.at[gi])
    def o_copy(gi):
        return pltpu.make_async_copy(out_buf.at[pl.ds(gi * U, U)], o_hbm.at[pl.ds(gi * U, U)], sem_o.at[gi])

    lane = jax.lax.broadcasted_iota(jnp.int32, (Sq, 128), 1)
    lo = lane < 64

    def stage_a(g):
        xg = x_buf[pl.ds(gi_of(g) * U, U)].reshape(M, D)
        q = jnp.dot(xg, wq_buf[hp_of(g) & 1], preferred_element_type=F32) * qscale
        res = []
        for u in range(U):
            qu = q[u * Sq:(u + 1) * Sq]
            q0 = qu[:, 0:128].astype(BF16)
            qm = qu[:, 128:256]
            q2 = qu[:, 256:384].astype(BF16)
            qmm = jnp.concatenate([jnp.where(lo, qm, 0.0), jnp.where(lo, 0.0, qm)], axis=0).astype(BF16)
            res.append((q0, qmm, q2))
        return res

    def stage_b(g, qs):
        slot = g & (NSLOT - 1)
        ps = g & 1
        for u in range(U):
            q0, qmm, q2 = qs[u]
            s0 = jnp.dot(q0, k_buf[slot, u, 0, 0:128, :], preferred_element_type=F32)
            km = jnp.concatenate([k_buf[slot, u, 0, 128:192, :], k_buf[slot, u, 1, 0:64, :]], axis=0)
            sm = jnp.dot(qmm, km, preferred_element_type=F32)
            s2 = jnp.dot(q2, k_buf[slot, u, 1, 64:192, :], preferred_element_type=F32)
            for h, s in ((0, s0 + sm[:Sq]), (1, s2 + sm[Sq:])):
                m = jnp.max(s, axis=-1, keepdims=True)
                p = jnp.exp2(s - m)
                l = jnp.sum(p, axis=-1, keepdims=True)
                p_buf[ps, u, h, 0:Sq, :] = p.astype(BF16)
                r_buf[ps, u, h] = jnp.broadcast_to(1.0 / l, (Sq, 128))

    def stage_c(g):
        slot = g & (NSLOT - 1)
        ps = g & 1
        os_ = []
        for u in range(U):
            ot0 = jax.lax.dot_general(v_buf[slot, u, 0], p_buf[ps, u, 0], NT, preferred_element_type=F32)
            ot1 = jax.lax.dot_general(v_buf[slot, u, 1], p_buf[ps, u, 1], NT, preferred_element_type=F32)
            t = jnp.concatenate([ot0, ot1], axis=0).T[:Sq]
            r0 = r_buf[ps, u, 0]
            r1 = r_buf[ps, u, 1]
            o = jnp.concatenate([t[:, 0:128] * r0, t[:, 128:256] * jnp.where(lo, r0, r1), t[:, 256:384] * r1], axis=1)
            os_.append(o.astype(BF16))
        return jnp.concatenate(os_, axis=0) if U > 1 else os_[0]

    def stage_d(g, o):
        rows = pl.ds(pl.multiple_of(gi_of(g) * M, 16), M)
        acc[rows, :] += jnp.dot(o, wo_buf[hp_of(g) & 1], preferred_element_type=F32)

    def stage_out(g):
        gi = gi_of(g)
        rows = pl.ds(pl.multiple_of(gi * M, 16), M)
        @pl.when(hp_of(g) == NP - 1)
        def _():
            out_buf[pl.ds(gi * U, U)] = acc[rows, :].astype(BF16).reshape(U, Sq, D)
            o_copy(gi).start()

    def issue(g):
        gk = g + NSLOT
        @pl.when(gk < NG)
        def _():
            k_copy(gk).start()
        gv = g + NSLOT - 1
        @pl.when(gv < NG)
        def _():
            v_copy(gv).start()
        hp = hp_of(g)
        gi = gi_of(g)
        @pl.when(jnp.logical_and(gi == 0, hp + 1 < NP))
        def _():
            wq_copy(hp + 1).start()
            wo_copy(hp + 1).start()

    x_copy(0).start()
    wq_copy(0).start()
    k_copy(0).start()
    acc[...] = jnp.zeros_like(acc)
    p_buf[...] = jnp.zeros_like(p_buf)
    x_copy(0).wait()
    wq_copy(0).wait()
    for gi in range(1, GP): x_copy(gi).start()
    v_copy(0).start()
    wo_copy(0).start()
    qs0 = stage_a(0)
    k_copy(0).wait()
    for g in range(1, NSLOT):
        k_copy(g).start()
        if g < NSLOT - 1:
            v_copy(g).start()
    stage_b(0, qs0)
    for gi in range(1, GP): x_copy(gi).wait()
    issue(0)

    def body(g, carry):
        hp = hp_of(g)
        gi = gi_of(g)
        @pl.when(gi == 0)
        def _():
            wq_copy(hp).wait()
        @pl.when(gi_of(g - 1) == 0)
        def _():
            wo_copy(hp_of(g - 1)).wait()
        k_copy(g).wait()
        v_copy(g - 1).wait()
        qs = stage_a(g)
        o = stage_c(g - 1)
        stage_b(g, qs)
        stage_d(g - 1, o)
        issue(g)
        stage_out(g - 1)
        return carry

    jax.lax.fori_loop(1, NG, body, 0)
    v_copy(NG - 1).wait()
    stage_d(NG - 1, stage_c(NG - 1))
    stage_out(NG - 1)
    for gi in range(GP): o_copy(gi).wait()


@jax.jit
def pallas_standalone__mha_block_cached__near_ridge_kernel(x, k_cache, v_cache, wq, wo):
    B, Sq, D = x.shape
    _, H, Sk, Dh = k_cache.shape
    kt = k_cache.transpose(0, 1, 3, 2)
    vt = v_cache.transpose(0, 1, 3, 2)
    W = 2 * Dh
    GP = B // U
    any_spec = pl.BlockSpec(memory_space=pl.ANY)
    return pl.pallas_call(
        functools.partial(_kernel, U=U, NSLOT=NSLOT),
        in_specs=[any_spec] * 5,
        out_specs=any_spec,
        out_shape=jax.ShapeDtypeStruct((B, Sq, D), x.dtype),
        scratch_shapes=[
            pltpu.VMEM((B, Sq, D), BF16),
            pltpu.VMEM((2, D, W), BF16),
            pltpu.VMEM((2, W, D), BF16),
            pltpu.VMEM((NSLOT, U, 2, Dh, Sk), BF16),
            pltpu.VMEM((NSLOT, U, 2, Dh, Sk), BF16),
            pltpu.VMEM((2, U, 2, 128, Sk), BF16),
            pltpu.VMEM((2, U, 2, Sq, 128), F32),
            pltpu.VMEM((B * Sq, D), F32),
            pltpu.VMEM((B, Sq, D), BF16),
            pltpu.SemaphoreType.DMA((GP,)),
            pltpu.SemaphoreType.DMA((2,)),
            pltpu.SemaphoreType.DMA((2,)),
            pltpu.SemaphoreType.DMA((NSLOT,)),
            pltpu.SemaphoreType.DMA((NSLOT,)),
            pltpu.SemaphoreType.DMA((GP,)),
        ],
        compiler_params=pltpu.CompilerParams(vmem_limit_bytes=100 * 1024 * 1024, disable_bounds_checks=True),
    )(x, kt, vt, wq, wo)
```

```python
import functools
import jax
import jax.numpy as jnp
from jax.experimental import pallas as pl
from jax.experimental.pallas import tpu as pltpu

U = 2
NSLOT = 4
LOG2E = 1.4426950408889634
F32 = jnp.float32
BF16 = jnp.bfloat16
NT = (((1,), (1,)), ((), ()))


def _log2(n):
    r = n.bit_length() - 1
    assert 1 << r == n
    return r


def _kernel(x_hbm, kt_hbm, vt_hbm, wq_hbm, wo_hbm, o_hbm,
            x_buf, wq_buf, wo_buf, k_buf, v_buf, q_buf, p_buf, r_buf, acc, out_buf,
            sem_x, sem_wq, sem_wo, sem_k, sem_v, sem_o, *, U, NSLOT):
    B, Sq, D = x_hbm.shape
    _, H, Dh, Sk = kt_hbm.shape
    NP = H // 2
    GP = B // U
    NG = NP * GP
    LGP = _log2(GP)
    M = U * Sq
    W = 2 * Dh
    qscale = (Dh ** -0.5) * LOG2E

    def hp_of(g): return g >> LGP
    def gi_of(g): return g & (GP - 1)

    def kv_copy(hbm, buf, sem, g):
        slot = g & (NSLOT - 1)
        return pltpu.make_async_copy(hbm.at[pl.ds(gi_of(g) * U, U), pl.ds(2 * hp_of(g), 2)], buf.at[slot], sem.at[slot])

    def k_copy(g): return kv_copy(kt_hbm, k_buf, sem_k, g)
    def v_copy(g): return kv_copy(vt_hbm, v_buf, sem_v, g)
    def wq_copy(hp):
        return pltpu.make_async_copy(wq_hbm.at[:, pl.ds(hp * W, W)], wq_buf.at[hp & 1], sem_wq.at[hp & 1])
    def wo_copy(hp):
        return pltpu.make_async_copy(wo_hbm.at[pl.ds(hp * W, W), :], wo_buf.at[hp & 1], sem_wo.at[hp & 1])
    def x_copy(gi):
        return pltpu.make_async_copy(x_hbm.at[pl.ds(gi * U, U)], x_buf.at[pl.ds(gi * U, U)], sem_x.at[gi])
    def o_copy(gi):
        return pltpu.make_async_copy(out_buf.at[pl.ds(gi * U, U)], o_hbm.at[pl.ds(gi * U, U)], sem_o.at[gi])

    def ol_copy(u):
        b = B - U + u
        return pltpu.make_async_copy(out_buf.at[b], o_hbm.at[b], sem_o.at[GP - 1 + u])

    lane = jax.lax.broadcasted_iota(jnp.int32, (Sq, 128), 1)
    lo = lane < 64

    def stage_a(g):
        hp = hp_of(g)
        gi = gi_of(g)
        xg = x_buf[pl.ds(gi * U, U)].reshape(M, D)
        q = jnp.dot(xg, wq_buf[hp & 1], preferred_element_type=F32) * qscale
        for u in range(U):
            qu = q[u * Sq:(u + 1) * Sq]
            qm = qu[:, 128:256]
            q_buf[hp & 1, gi, u, 0 * Sq:1 * Sq, :] = qu[:, 0:128].astype(BF16)
            q_buf[hp & 1, gi, u, 1 * Sq:2 * Sq, :] = jnp.where(lo, qm, 0.0).astype(BF16)
            q_buf[hp & 1, gi, u, 2 * Sq:3 * Sq, :] = jnp.where(lo, 0.0, qm).astype(BF16)
            q_buf[hp & 1, gi, u, 3 * Sq:4 * Sq, :] = qu[:, 256:384].astype(BF16)

    def stage_b(g):
        slot = g & (NSLOT - 1)
        ps = g & 1
        hp = hp_of(g)
        gi = gi_of(g)
        for u in range(U):
            q0 = q_buf[hp & 1, gi, u, 0 * Sq:1 * Sq, :]
            qmm = q_buf[hp & 1, gi, u, 1 * Sq:3 * Sq, :]
            q2 = q_buf[hp & 1, gi, u, 3 * Sq:4 * Sq, :]
            s0 = jnp.dot(q0, k_buf[slot, u, 0, 0:128, :], preferred_element_type=F32)
            km = jnp.concatenate([k_buf[slot, u, 0, 128:192, :], k_buf[slot, u, 1, 0:64, :]], axis=0)
            sm = jnp.dot(qmm, km, preferred_element_type=F32)
            s2 = jnp.dot(q2, k_buf[slot, u, 1, 64:192, :], preferred_element_type=F32)
            for h, s in ((0, s0 + sm[:Sq]), (1, s2 + sm[Sq:])):
                m = jnp.max(s, axis=-1, keepdims=True)
                p = jnp.exp2(s - m)
                l = jnp.sum(p, axis=-1, keepdims=True)
                p_buf[ps, u, h, 0:Sq, :] = p.astype(BF16)
                r_buf[ps, u, h] = jnp.broadcast_to(1.0 / l, (Sq, 128))

    def stage_c_item(g, u):
        slot = g & (NSLOT - 1)
        ps = g & 1
        ot0 = jax.lax.dot_general(v_buf[slot, u, 0], p_buf[ps, u, 0], NT, preferred_element_type=F32)
        ot1 = jax.lax.dot_general(v_buf[slot, u, 1], p_buf[ps, u, 1], NT, preferred_element_type=F32)
        t = jnp.concatenate([ot0, ot1], axis=0).T[:Sq]
        r0 = r_buf[ps, u, 0]
        r1 = r_buf[ps, u, 1]
        o = jnp.concatenate([t[:, 0:128] * r0, t[:, 128:256] * jnp.where(lo, r0, r1), t[:, 256:384] * r1], axis=1)
        return o.astype(BF16)

    def stage_c(g):
        os_ = [stage_c_item(g, u) for u in range(U)]
        return jnp.concatenate(os_, axis=0) if U > 1 else os_[0]

    def stage_d(g, o):
        rows = pl.ds(pl.multiple_of(gi_of(g) * M, 16), M)
        acc[rows, :] += jnp.dot(o, wo_buf[hp_of(g) & 1], preferred_element_type=F32)

    def stage_d_final(g, o):
        gi = gi_of(g)
        rows = pl.ds(pl.multiple_of(gi * M, 16), M)
        res = acc[rows, :] + jnp.dot(o, wo_buf[hp_of(g) & 1], preferred_element_type=F32)
        out_buf[pl.ds(gi * U, U)] = res.astype(BF16).reshape(U, Sq, D)

    def issue(g, weights=True):
        gk = g + NSLOT
        @pl.when(gk < NG)
        def _():
            k_copy(gk).start()
        gv = g + NSLOT - 1
        @pl.when(gv < NG)
        def _():
            v_copy(gv).start()
        if not weights:
            return
        hp = hp_of(g)
        gi = gi_of(g)
        @pl.when(jnp.logical_and(gi == 0, hp + 2 < NP))
        def _():
            wq_copy(hp + 2).start()
        @pl.when(jnp.logical_and(gi == 0, hp + 1 < NP))
        def _():
            wo_copy(hp + 1).start()

    def waits(g):
        @pl.when(gi_of(g - 1) == 0)
        def _():
            wo_copy(hp_of(g - 1)).wait()
        k_copy(g).wait()
        v_copy(g - 1).wait()

    x_copy(0).start()
    wq_copy(0).start()
    for gi in range(1, GP): x_copy(gi).start()
    acc[...] = jnp.zeros_like(acc)
    p_buf[:, :, :, Sq:, :] = jnp.zeros((2, U, 2, 128 - Sq, Sk), BF16)
    x_copy(0).wait()
    wq_copy(0).wait()
    k_copy(0).start()
    wq_copy(1).start()
    v_copy(0).start()
    wo_copy(0).start()
    stage_a(0)
    for gi in range(1, GP):
        x_copy(gi).wait()
    for g in range(1, NSLOT):
        k_copy(g).start()
        if g < NSLOT - 1:
            v_copy(g).start()
    for gi in range(1, GP):
        stage_a(gi)
    k_copy(0).wait()
    wq_copy(1).wait()
    stage_b(0)
    stage_a(GP)
    issue(0)

    def body(g, carry):
        @pl.when(gi_of(g) == 0)
        def _():
            wq_copy(hp_of(g) + 1).wait()
        waits(g)
        stage_a(g + GP)
        o = stage_c(g - 1)
        stage_b(g)
        stage_d(g - 1, o)
        issue(g)
        return carry

    jax.lax.fori_loop(1, NG - GP, body, 0)

    g = NG - GP
    waits(g)
    o = stage_c(g - 1)
    stage_b(g)
    stage_d(g - 1, o)
    issue(g, weights=False)

    def body_last(g, carry):
        waits(g)
        o = stage_c(g - 1)
        stage_b(g)
        stage_d_final(g - 1, o)
        return carry

    jax.lax.fori_loop(NG - GP + 1, NG, body_last, 0)
    g = NG - 1
    v_copy(g).wait()
    for gi in range(GP - 1): o_copy(gi).start()
    os_ = [stage_c_item(g, u) for u in range(U)]
    for u in range(U):
        b = B - U + u
        res = acc[b * Sq:(b + 1) * Sq, :] + jnp.dot(os_[u], wo_buf[(NP - 1) & 1], preferred_element_type=F32)
        out_buf[b] = res.astype(BF16)
        ol_copy(u).start()
    for gi in range(GP - 1): o_copy(gi).wait()
    for u in range(U): ol_copy(u).wait()


@jax.jit
def pallas_standalone__mha_block_cached__near_ridge_kernel(x, k_cache, v_cache, wq, wo):
    B, Sq, D = x.shape
    _, H, Sk, Dh = k_cache.shape
    kt = k_cache.transpose(0, 1, 3, 2)
    vt = v_cache.transpose(0, 1, 3, 2)
    W = 2 * Dh
    GP = B // U
    any_spec = pl.BlockSpec(memory_space=pl.ANY)
    return pl.pallas_call(
        functools.partial(_kernel, U=U, NSLOT=NSLOT),
        in_specs=[any_spec] * 5,
        out_specs=any_spec,
        out_shape=jax.ShapeDtypeStruct((B, Sq, D), x.dtype),
        scratch_shapes=[
            pltpu.VMEM((B, Sq, D), BF16),
            pltpu.VMEM((2, D, W), BF16),
            pltpu.VMEM((2, W, D), BF16),
            pltpu.VMEM((NSLOT, U, 2, Dh, Sk), BF16),
            pltpu.VMEM((NSLOT, U, 2, Dh, Sk), BF16),
            pltpu.VMEM((2, GP, U, 4 * Sq, 128), BF16),
            pltpu.VMEM((2, U, 2, 128, Sk), BF16),
            pltpu.VMEM((2, U, 2, Sq, 128), F32),
            pltpu.VMEM((B * Sq, D), F32),
            pltpu.VMEM((B, Sq, D), BF16),
            pltpu.SemaphoreType.DMA((GP,)),
            pltpu.SemaphoreType.DMA((2,)),
            pltpu.SemaphoreType.DMA((2,)),
            pltpu.SemaphoreType.DMA((NSLOT,)),
            pltpu.SemaphoreType.DMA((NSLOT,)),
            pltpu.SemaphoreType.DMA((GP - 1 + U,)),
        ],
        compiler_params=pltpu.CompilerParams(vmem_limit_bytes=100 * 1024 * 1024, disable_bounds_checks=True),
    )(x, kt, vt, wq, wo)
```

```python
import jax
import jax.numpy as jnp
from jax.experimental import pallas as pl
from jax.experimental.pallas import tpu as pltpu

U = 2
NSLOT = 4
LANES = 128
LOG2E = 1.4426950408889634
F32 = jnp.float32
BF16 = jnp.bfloat16
NT = (((1,), (1,)), ((), ()))


def _log2(n):
    r = n.bit_length() - 1
    assert 1 << r == n
    return r


def _kernel(x_hbm, kt_hbm, vt_hbm, wq_hbm, wo_hbm, o_hbm,
            x_buf, wq_buf, wo_buf, k_buf, v_buf, q_buf, p_buf, r_buf, acc, out_buf,
            sem_x, sem_wq, sem_wo, sem_k, sem_v, sem_o):
    B, Sq, D = x_hbm.shape
    _, H, Dh, Sk = kt_hbm.shape
    NP = H // 2
    GP = B // U
    NG = NP * GP
    LGP = _log2(GP)
    M = U * Sq
    W = 2 * Dh
    HALF = Dh - LANES
    qscale = (Dh ** -0.5) * LOG2E
    assert NSLOT == GP == 4 and NP >= 3 and Dh == 192 and Sq <= LANES

    def hp_of(g): return g >> LGP
    def gi_of(g): return g & (GP - 1)
    def slot_of(g): return g & (NSLOT - 1)

    def kv_copy(hbm, buf, sem, g):
        return pltpu.make_async_copy(hbm.at[pl.ds(gi_of(g) * U, U), pl.ds(2 * hp_of(g), 2)],
                                     buf.at[slot_of(g)], sem.at[slot_of(g)])

    def k_copy(g): return kv_copy(kt_hbm, k_buf, sem_k, g)
    def v_copy(g): return kv_copy(vt_hbm, v_buf, sem_v, g)

    def wq_copy(hp):
        return pltpu.make_async_copy(wq_hbm.at[:, pl.ds(hp * W, W)], wq_buf.at[hp & 1], sem_wq.at[hp & 1])

    def wo_copy(hp):
        return pltpu.make_async_copy(wo_hbm.at[pl.ds(hp * W, W), :], wo_buf.at[hp & 1], sem_wo.at[hp & 1])

    def x_copy(gi):
        return pltpu.make_async_copy(x_hbm.at[pl.ds(gi * U, U)], x_buf.at[pl.ds(gi * U, U)], sem_x.at[gi])

    def o_copy(gi):
        return pltpu.make_async_copy(out_buf.at[pl.ds(gi * U, U)], o_hbm.at[pl.ds(gi * U, U)], sem_o.at[gi])

    def o_item_copy(u):
        b = B - U + u
        return pltpu.make_async_copy(out_buf.at[b], o_hbm.at[b], sem_o.at[GP - 1 + u])

    lo = jax.lax.broadcasted_iota(jnp.int32, (Sq, LANES), 1) < HALF

    def stage_a(g):
        hp = hp_of(g)
        gi = gi_of(g)
        xg = x_buf[pl.ds(gi * U, U)].reshape(M, D)
        q = jnp.dot(xg, wq_buf[hp & 1], preferred_element_type=F32) * qscale
        for u in range(U):
            qu = q[u * Sq:(u + 1) * Sq]
            qm = qu[:, LANES:2 * LANES]
            q_buf[hp & 1, gi, u, 0 * Sq:1 * Sq, :] = qu[:, 0:LANES].astype(BF16)
            q_buf[hp & 1, gi, u, 1 * Sq:2 * Sq, :] = jnp.where(lo, qm, 0.0).astype(BF16)
            q_buf[hp & 1, gi, u, 2 * Sq:3 * Sq, :] = jnp.where(lo, 0.0, qm).astype(BF16)
            q_buf[hp & 1, gi, u, 3 * Sq:4 * Sq, :] = qu[:, 2 * LANES:3 * LANES].astype(BF16)

    def stage_b(g):
        slot = slot_of(g)
        ps = g & 1
        hp = hp_of(g)
        gi = gi_of(g)
        for u in range(U):
            q0 = q_buf[hp & 1, gi, u, 0 * Sq:1 * Sq, :]
            qmm = q_buf[hp & 1, gi, u, 1 * Sq:3 * Sq, :]
            q2 = q_buf[hp & 1, gi, u, 3 * Sq:4 * Sq, :]
            s0 = jnp.dot(q0, k_buf[slot, u, 0, 0:LANES, :], preferred_element_type=F32)
            km = jnp.concatenate([k_buf[slot, u, 0, LANES:Dh, :], k_buf[slot, u, 1, 0:HALF, :]], axis=0)
            sm = jnp.dot(qmm, km, preferred_element_type=F32)
            s2 = jnp.dot(q2, k_buf[slot, u, 1, HALF:Dh, :], preferred_element_type=F32)
            for h, s in ((0, s0 + sm[:Sq]), (1, s2 + sm[Sq:])):
                m = jnp.max(s, axis=-1, keepdims=True)
                p = jnp.exp2(s - m)
                l = jnp.sum(p, axis=-1, keepdims=True)
                p_buf[ps, u, h, 0:Sq, :] = p.astype(BF16)
                r_buf[ps, u, h] = jnp.broadcast_to(1.0 / l, (Sq, LANES))

    def stage_c_item(g, u):
        slot = slot_of(g)
        ps = g & 1
        ot0 = jax.lax.dot_general(v_buf[slot, u, 0], p_buf[ps, u, 0], NT, preferred_element_type=F32)
        ot1 = jax.lax.dot_general(v_buf[slot, u, 1], p_buf[ps, u, 1], NT, preferred_element_type=F32)
        t = jnp.concatenate([ot0, ot1], axis=0).T[:Sq]
        r0 = r_buf[ps, u, 0]
        r1 = r_buf[ps, u, 1]
        o = jnp.concatenate([t[:, 0:LANES] * r0,
                             t[:, LANES:2 * LANES] * jnp.where(lo, r0, r1),
                             t[:, 2 * LANES:3 * LANES] * r1], axis=1)
        return o.astype(BF16)

    def stage_c(g):
        return jnp.concatenate([stage_c_item(g, u) for u in range(U)], axis=0)

    def group_rows(g):
        return pl.ds(pl.multiple_of(gi_of(g) * M, 16), M)

    def stage_d(g, o):
        acc[group_rows(g), :] += jnp.dot(o, wo_buf[hp_of(g) & 1], preferred_element_type=F32)

    def stage_d_final(g, o):
        res = acc[group_rows(g), :] + jnp.dot(o, wo_buf[hp_of(g) & 1], preferred_element_type=F32)
        out_buf[pl.ds(gi_of(g) * U, U)] = res.astype(BF16).reshape(U, Sq, D)

    def issue(g, weights=True):
        gk = g + NSLOT
        @pl.when(gk < NG)
        def _():
            k_copy(gk).start()
        gv = g + NSLOT - 1
        @pl.when(gv < NG)
        def _():
            v_copy(gv).start()
        if not weights:
            return
        hp = hp_of(g)
        gi = gi_of(g)
        @pl.when(jnp.logical_and(gi == 0, hp + 2 < NP))
        def _():
            wq_copy(hp + 2).start()
        @pl.when(jnp.logical_and(gi == 0, hp + 1 < NP))
        def _():
            wo_copy(hp + 1).start()

    def waits(g):
        @pl.when(gi_of(g - 1) == 0)
        def _():
            wo_copy(hp_of(g - 1)).wait()
        k_copy(g).wait()
        v_copy(g - 1).wait()

    x_copy(0).start()
    wq_copy(0).start()
    for gi in range(1, GP):
        x_copy(gi).start()
    acc[...] = jnp.zeros_like(acc)
    p_buf[:, :, :, Sq:, :] = jnp.zeros((2, U, 2, LANES - Sq, Sk), BF16)
    x_copy(0).wait()
    wq_copy(0).wait()
    k_copy(0).start()
    wq_copy(1).start()
    v_copy(0).start()
    wo_copy(0).start()
    stage_a(0)
    for gi in range(1, GP):
        x_copy(gi).wait()
    for g in range(1, NSLOT):
        k_copy(g).start()
        if g < NSLOT - 1:
            v_copy(g).start()
    for gi in range(1, GP):
        stage_a(gi)
    k_copy(0).wait()
    wq_copy(1).wait()
    stage_b(0)
    stage_a(GP)
    issue(0)

    def body(g, carry):
        @pl.when(gi_of(g) == 0)
        def _():
            wq_copy(hp_of(g) + 1).wait()
        waits(g)
        stage_a(g + GP)
        o = stage_c(g - 1)
        stage_b(g)
        stage_d(g - 1, o)
        issue(g)
        return carry

    jax.lax.fori_loop(1, NG - GP, body, 0)

    g = NG - GP
    waits(g)
    o = stage_c(g - 1)
    stage_b(g)
    stage_d(g - 1, o)
    issue(g, weights=False)

    def body_last(g, carry):
        waits(g)
        o = stage_c(g - 1)
        stage_b(g)
        stage_d_final(g - 1, o)
        return carry

    jax.lax.fori_loop(NG - GP + 1, NG, body_last, 0)

    g = NG - 1
    v_copy(g).wait()
    for gi in range(GP - 1):
        o_copy(gi).start()
    os_ = [stage_c_item(g, u) for u in range(U)]
    for u in range(U):
        b = B - U + u
        res = acc[b * Sq:(b + 1) * Sq, :] + jnp.dot(os_[u], wo_buf[(NP - 1) & 1], preferred_element_type=F32)
        out_buf[b] = res.astype(BF16)
        o_item_copy(u).start()
    for gi in range(GP - 1):
        o_copy(gi).wait()
    for u in range(U):
        o_item_copy(u).wait()


@jax.jit
def pallas_standalone__mha_block_cached__near_ridge_kernel(
    x: jax.Array,
    k_cache: jax.Array,
    v_cache: jax.Array,
    wq: jax.Array,
    wo: jax.Array,
):
    B, Sq, D = x.shape
    _, H, Sk, Dh = k_cache.shape
    kt = k_cache.transpose(0, 1, 3, 2)
    vt = v_cache.transpose(0, 1, 3, 2)
    W = 2 * Dh
    GP = B // U
    any_spec = pl.BlockSpec(memory_space=pl.ANY)
    return pl.pallas_call(
        _kernel,
        in_specs=[any_spec] * 5,
        out_specs=any_spec,
        out_shape=jax.ShapeDtypeStruct((B, Sq, D), x.dtype),
        scratch_shapes=[
            pltpu.VMEM((B, Sq, D), BF16),
            pltpu.VMEM((2, D, W), BF16),
            pltpu.VMEM((2, W, D), BF16),
            pltpu.VMEM((NSLOT, U, 2, Dh, Sk), BF16),
            pltpu.VMEM((NSLOT, U, 2, Dh, Sk), BF16),
            pltpu.VMEM((2, GP, U, 4 * Sq, LANES), BF16),
            pltpu.VMEM((2, U, 2, LANES, Sk), BF16),
            pltpu.VMEM((2, U, 2, Sq, LANES), F32),
            pltpu.VMEM((B * Sq, D), F32),
            pltpu.VMEM((B, Sq, D), BF16),
            pltpu.SemaphoreType.DMA((GP,)),
            pltpu.SemaphoreType.DMA((2,)),
            pltpu.SemaphoreType.DMA((2,)),
            pltpu.SemaphoreType.DMA((NSLOT,)),
            pltpu.SemaphoreType.DMA((NSLOT,)),
            pltpu.SemaphoreType.DMA((GP - 1 + U,)),
        ],
        compiler_params=pltpu.CompilerParams(
            vmem_limit_bytes=64 * 1024 * 1024,
            disable_bounds_checks=True,
        ),
    )(x, kt, vt, wq, wo)
```
